```python
import jax
import jax.numpy as jnp

def _softmax(x, axis=-1):
    return jax.nn.softmax(x, axis=axis)
def _gelu(x):
    return jax.nn.gelu(x, approximate=True)
def _silu(x):
    return jax.nn.silu(x)
def _sigmoid(x):
    return jax.nn.sigmoid(x)
def _layernorm(x, axis=-1, eps=1e-5):
    m = jnp.mean(x, axis=axis, keepdims=True)
    v = jnp.var(x, axis=axis, keepdims=True)
    return (x - m) / jnp.sqrt(v + eps)
def _scatter_add(tgt, idx, src, axis=0):
    return tgt.at[idx].add(src)
def _segment_sum(src, seg, n):
    return jax.ops.segment_sum(src, seg, n)
class _Rng:
    def __init__(self, key):
        self._k = key
    def _next(self):
        self._k, sub = jax.random.split(self._k)
        return sub
    def normal(self, shape):
        return jax.random.normal(self._next(), shape, dtype=jnp.bfloat16)
    def randint(self, lo, hi, shape):
        return jax.random.randint(self._next(), shape, lo, hi, dtype=jnp.int32)
    def uniform(self, shape, lo=0.0, hi=1.0):
        return jax.random.uniform(self._next(), shape, jnp.bfloat16, lo, hi)
    def permutation(self, n):
        return jax.random.permutation(self._next(), n)


kernel_name = 'standalone__channel_attn_se__vision'

def _fwd_setup_inputs():
    _rng = _Rng(jax.random.key(int.from_bytes(__import__("os").urandom(4), "little")))
    _w = (lambda a: (lambda t: t.astype(jnp.bfloat16) if jnp.issubdtype(t.dtype, jnp.floating) else t)(jnp.asarray(a)))
    H = W = 384
    C = 96
    r = max(C // 16, 4)
    return {
        "x": _w((lambda *s: _rng.normal(s) * 0.05)(1, H, W, C)),
        "w_down": _w((lambda *s: _rng.normal(s) * 0.05)(C, r)),
        "w_up": _w((lambda *s: _rng.normal(s) * 0.05)(r, C)),
    }

def _fwd_reference(x, w_down, w_up):
    s = x.mean(axis=(1, 2))
    h = _silu(jnp.einsum('bc,cr->br', s, w_down))
    g = _sigmoid(jnp.einsum('br,rc->bc', h, w_up))
    return x * g[:, None, None, :]


def setup_inputs():
    _inp = _fwd_setup_inputs()
    _gk = jax.random.fold_in(jax.random.key(int.from_bytes(__import__("os").urandom(4), "little")), 2**31 - 1)
    _shapes = [[1, 384, 384, 96]]
    _dtypes = ['bfloat16']
    _gks = jax.random.split(_gk, len(_shapes))
    _gs = [jax.random.normal(k, s, dtype=jnp.dtype(d)) * 0.05 for k, s, d in zip(_gks, _shapes, _dtypes)]
    _inp["grad_out"] = _gs[0]
    return _inp

def reference(x, w_down, w_up, grad_out):
    _const = dict()
    def _f(*_d):
        return _fwd_reference(**{'x': _d[0], 'w_down': _d[1], 'w_up': _d[2], **_const})
    _out, _vjp = jax.vjp(_f, x, w_down, w_up)
    _grads = _vjp(grad_out)
    _out0 = jnp.asarray(_out)
    return (_out0, *[jnp.asarray(_g) for _g in _grads])
```

```python
import jax
import jax.numpy as jnp
from jax import lax
import jax.experimental.pallas as pl
import jax.experimental.pallas.tpu as pltpu

LANES = 128
SUB = 8

SEG = 4096
READ_ROWS = 16
WRITE_ROWS = 16
FIRST_ROWS = 64
SKEW = 26
SETTLE = 36
LEAD = 13
WRITE_BLOCKS = (6, 7, 7, 7)
HIGH_SETS = ((0, 0), (1, 0), (1, 1))
LOW_SETS = ((0, 1), (0, 2), (1, 2))


def _se_kernel_factory(H, W, C):
    WB = W // LANES
    CB = C // SUB
    ROWS = C * WB
    NSEG = H * ROWS // SEG
    SET_SEGS = NSEG // 3
    HT = H // 3
    NR = SEG // READ_ROWS
    inv_n = 1.0 / (H * W)
    assert W % LANES == 0 and C % (2 * SUB) == 0
    assert HT * 3 == H and HT * ROWS == SET_SEGS * SEG and sum(WRITE_BLOCKS) == NSEG

    blocks = [(a, sum(WRITE_BLOCKS[:k]), n)
              for a in range(2) for k, n in enumerate(WRITE_BLOCKS)]

    def rows_needed(b):
        _, s0, n = blocks[b]
        return -(-(s0 + n) * SEG // ROWS)

    def kernel(x_hbm, go_hbm, wd_hbm, wu_hbm, out_hbm, dx_hbm, dwd_hbm, dwu_hbm,
               xb, gb, wd_v, wu_v, dwd_v, dwu_v, rsem, wsem, ssem):
        seg_v = (xb.reshape(NSEG, SEG, LANES), gb.reshape(NSEG, SEG, LANES))
        src_h = (x_hbm, go_hbm)
        dst_h = (out_hbm, dx_hbm)

        def aligned(v):
            return v if isinstance(v, int) else pl.multiple_of(v, 2 * SUB)

        def read_copy(st, j, n=1, sem=None):
            a, third = st
            idx = (pl.ds(third * SET_SEGS, SET_SEGS),
                   pl.ds(aligned(j * READ_ROWS), n * READ_ROWS))
            sem = 3 * a + third if sem is None else sem
            return pltpu.make_async_copy(src_h[a].at[idx], seg_v[a].at[idx], rsem.at[sem])

        def read_steps(i0, i1, body=None, carry=0):
            cuts = {i0, i1} | {p * NR for p in range(3)} | {p * NR - SKEW for p in range(3)}
            cuts = sorted(c for c in cuts if i0 <= c <= i1)
            assert body is None or len(cuts) == 2
            for lo, hi in zip(cuts[:-1], cuts[1:]):
                ph, pw = lo // NR, (lo + SKEW) // NR

                def step(i, c, ph=ph, pw=pw):
                    read_copy(HIGH_SETS[ph], i - ph * NR).start(priority=0)
                    read_copy(LOW_SETS[pw], i + SKEW - pw * NR).start(priority=1)
                    return c if body is None else body(i - i0, c)

                carry = lax.fori_loop(lo, hi, step, carry)
            return carry

        last_sets = (HIGH_SETS[2], LOW_SETS[2])
        shared = NR - SKEW // 2
        drain = [(last_sets[u % 2], shared + u // 2) for u in range(SKEW)]
        marker = drain[SKEW - LEAD]
        marker_copy = read_copy(*marker, sem=6)

        def read_drain():
            for u, piece in enumerate(drain):
                read_copy(last_sets[0], shared - SKEW + u).start(priority=0)
                (marker_copy if piece == marker else read_copy(*piece)).start(priority=1)

        def write_block(b, rows, body=None, h0=0, nh=0, carry=0):
            a, s0, n = blocks[b]
            steps = nh if body is not None else SEG // rows
            per = SEG // rows // steps
            assert per * steps * rows == SEG

            def step(j, c):
                for u in range(per):
                    idx = (pl.ds(s0, n), pl.ds(aligned((j * per + u) * rows), rows))
                    pltpu.make_async_copy(seg_v[a].at[idx], dst_h[a].at[idx], wsem.at[a]).start()
                return c if body is None else body(h0 + j, c)

            return lax.fori_loop(0, steps, step, carry)

        slab = 2 * SUB * WB
        slabs = [(2 * k, pl.ds(k * slab, slab)) for k in range(CB // 2)]

        def tiles(v, half):
            return [v[(half * WB + i) * SUB:(half * WB + i + 1) * SUB] for i in range(WB)]

        def tile_sum(v, half):
            ts = tiles(v, half)
            s = ts[0]
            for t in ts[1:]:
                s = s + t
            return s

        def repeat(body, h0, n):
            def f(i, c):
                for u in range(n):
                    c = body(h0 + i * n + u, c)
                return c
            return f

        def diag():
            return (lax.broadcasted_iota(jnp.int32, (C, C), 0)
                    == lax.broadcasted_iota(jnp.int32, (C, C), 1))

        def acc_to_row(acc):
            col = jnp.sum(jnp.concatenate(acc, axis=0), axis=1, keepdims=True)
            return jnp.sum(jnp.where(diag(), col, 0.0), axis=0, keepdims=True)

        def row_to_tiles(row):
            col = jnp.sum(jnp.where(diag(), row, 0.0), axis=1, keepdims=True)
            full = jnp.broadcast_to(col, (C, LANES))
            return tuple(full[i * SUB:(i + 1) * SUB] for i in range(CB))

        zeros = tuple(jnp.zeros((SUB, LANES), jnp.float32) for _ in range(CB))

        def sum_x(h, acc):
            acc = list(acc)
            for cb, rows in slabs:
                v = xb[h, rows, :].astype(jnp.float32)
                for half in range(2):
                    acc[cb + half] = acc[cb + half] + tile_sum(v, half)
            return tuple(acc)

        for j in range(SKEW):
            read_copy(LOW_SETS[0], j).start(priority=1)
        read_steps(0, NR)
        wd_copy = pltpu.make_async_copy(wd_hbm, wd_v, ssem.at[0])
        wu_copy = pltpu.make_async_copy(wu_hbm, wu_v, ssem.at[1])
        wd_copy.start()
        wu_copy.start()
        i = NR + SETTLE
        read_steps(NR, i)
        read_copy(HIGH_SETS[0], 0, NR).wait()
        read_copy(LOW_SETS[0], 0, NR).wait()
        acc = read_steps(i, i + HT, repeat(sum_x, 0, 2), zeros)
        read_steps(i + HT, 2 * NR + SETTLE)

        i = 2 * NR + SETTLE
        read_copy(HIGH_SETS[1], 0, NR).wait()
        read_copy(LOW_SETS[1], 0, NR).wait()
        acc = read_steps(i, i + HT // 4, repeat(sum_x, 2 * HT, 4), acc)
        i += HT // 4

        wd_copy.wait()
        wu_copy.wait()
        wd = wd_v[...].astype(jnp.float32)
        wu = wu_v[...].astype(jnp.float32)
        s_row = acc_to_row(acc) * inv_n
        z1 = jnp.sum(wd * s_row, axis=1, keepdims=True)
        sig1 = jax.nn.sigmoid(z1)
        hid = z1 * sig1
        gate = jax.nn.sigmoid(jnp.sum(wu * hid, axis=0, keepdims=True))
        gate_t = row_to_tiles(gate)

        def scale_x(h, acc):
            acc = list(acc)
            for cb, rows in slabs:
                xv = xb[h, rows, :].astype(jnp.float32)
                prod = xv * gb[h, rows, :].astype(jnp.float32)
                outs = []
                for half in range(2):
                    acc[cb + half] = acc[cb + half] + tile_sum(prod, half)
                    outs += [t * gate_t[cb + half] for t in tiles(xv, half)]
                xb[h, rows, :] = jnp.concatenate(outs, axis=0).astype(xb.dtype)
            return tuple(acc)

        acc = read_steps(i, i + HT, scale_x, zeros)
        read_steps(i + HT, 2 * NR + shared - SKEW)
        read_drain()

        h1, h2 = HT + HT // 2, 2 * HT + HT // 2
        assert rows_needed(0) <= HT and rows_needed(1) <= h1 and rows_needed(2) <= h2
        marker_copy.wait()
        write_block(0, FIRST_ROWS)
        for st in last_sets:
            read_copy(st, 0, NR - 1 if st == marker[0] else NR).wait()
        acc = lax.fori_loop(HT, h1, scale_x, acc)
        acc = write_block(1, WRITE_ROWS, scale_x, h1, h2 - h1, acc)
        acc = write_block(2, WRITE_ROWS, scale_x, h2, H - h2, acc)

        dz2 = acc_to_row(acc) * gate * (1.0 - gate)
        dwu_v[...] = (hid * dz2).astype(dwu_v.dtype)
        dh = jnp.sum(wu * dz2, axis=1, keepdims=True)
        dz1 = dh * (sig1 * (1.0 + z1 * (1.0 - sig1)))
        dwd_v[...] = (dz1 * s_row).astype(dwd_v.dtype)
        ds_t = row_to_tiles(jnp.sum(wd * dz1, axis=0, keepdims=True) * inv_n)
        dwd_copy = pltpu.make_async_copy(dwd_v, dwd_hbm, ssem.at[2])
        dwu_copy = pltpu.make_async_copy(dwu_v, dwu_hbm, ssem.at[3])
        dwd_copy.start()
        dwu_copy.start()

        def grad_x(h, c):
            for cb, rows in slabs:
                gv = gb[h, rows, :].astype(jnp.float32)
                outs = []
                for half in range(2):
                    outs += [t * gate_t[cb + half] + ds_t[cb + half] for t in tiles(gv, half)]
                gb[h, rows, :] = jnp.concatenate(outs, axis=0).astype(gb.dtype)
            return c

        assert len(blocks) == 8 and rows_needed(4) <= HT and rows_needed(5) <= 2 * HT
        write_block(3, WRITE_ROWS, grad_x, 0, HT)
        write_block(4, WRITE_ROWS, grad_x, HT, HT)
        write_block(5, WRITE_ROWS, grad_x, 2 * HT, HT)
        write_block(6, WRITE_ROWS)
        write_block(7, WRITE_ROWS)

        dwd_copy.wait()
        dwu_copy.wait()
        pltpu.make_async_copy(seg_v[0], out_hbm, wsem.at[0]).wait()
        pltpu.make_async_copy(seg_v[1], dx_hbm, wsem.at[1]).wait()

    return kernel


@jax.jit
def pallas_standalone__channel_attn_se__vision_kernel(
    x: jax.Array,
    w_down: jax.Array,
    w_up: jax.Array,
    grad_out: jax.Array,
):
    B, H, W, C = x.shape
    R = w_down.shape[1]
    assert B == 1
    WB = W // LANES
    rows = C * WB
    seg_shape = (H * rows // SEG, SEG, LANES)

    def to_segments(a):
        a = jnp.transpose(a, (0, 1, 3, 2)).reshape(H * C // SUB, SUB, WB, LANES)
        return jnp.transpose(a, (0, 2, 1, 3)).reshape(seg_shape)

    def from_segments(a):
        a = a.reshape(H * C // SUB, WB, SUB, LANES)
        a = jnp.transpose(a, (0, 2, 1, 3)).reshape(B, H, C, W)
        return jnp.transpose(a, (0, 1, 3, 2))

    any_spec = pl.BlockSpec(memory_space=pl.ANY)
    out, dx, dwd_t, dwu = pl.pallas_call(
        _se_kernel_factory(H, W, C),
        in_specs=[any_spec] * 4,
        out_specs=[any_spec] * 4,
        out_shape=[
            jax.ShapeDtypeStruct(seg_shape, x.dtype),
            jax.ShapeDtypeStruct(seg_shape, x.dtype),
            jax.ShapeDtypeStruct((R, C), w_down.dtype),
            jax.ShapeDtypeStruct((R, C), w_up.dtype),
        ],
        scratch_shapes=[
            pltpu.VMEM((H, rows, LANES), x.dtype),
            pltpu.VMEM((H, rows, LANES), grad_out.dtype),
            pltpu.VMEM((R, C), w_down.dtype),
            pltpu.VMEM((R, C), w_up.dtype),
            pltpu.VMEM((R, C), w_down.dtype),
            pltpu.VMEM((R, C), w_up.dtype),
            pltpu.SemaphoreType.DMA((7,)),
            pltpu.SemaphoreType.DMA((2,)),
            pltpu.SemaphoreType.DMA((4,)),
        ],
        compiler_params=pltpu.CompilerParams(
            vmem_limit_bytes=80 * 1024 * 1024,
            disable_semaphore_checks=True,
            disable_bounds_checks=True,
        ),
    )(to_segments(x), to_segments(grad_out), w_down.T, w_up)
    return from_segments(out), from_segments(dx), dwd_t.T, dwu
```

```python
import math

import jax
import jax.numpy as jnp
from jax import lax
import jax.experimental.pallas as pl
import jax.experimental.pallas.tpu as pltpu

LANES = 128
SUB = 8

SEG = 4096
PIECE = 16
SKEW = 26
SETTLE = 36
LEAD = 13
PRELOAD = 5
WRITE_BLOCKS = (6, 7, 7, 7)
HIGH_SETS = ((0, 0), (1, 0), (1, 1))
LOW_SETS = ((0, 1), (0, 2), (1, 2))


def _make_kernel(H, W, C):
    WB = W // LANES
    CB = C // SUB
    ROWS = C * WB
    NSEG = H * ROWS // SEG
    SET_SEGS = NSEG // 3
    CH = math.gcd(SEG, ROWS)
    NV = SEG // CH
    NP = SEG // PIECE
    assert W % LANES == 0 and C % SUB == 0 and 3 * SET_SEGS * SEG == H * ROWS
    assert SET_SEGS * CH == ROWS and CH % PIECE == 0 and PIECE % (2 * SUB) == 0
    assert sum(WRITE_BLOCKS) == NSEG and NV % 4 == 0
    inv_nv = pow(NV, -1, SET_SEGS)
    inv_n = 1.0 / (H * W)

    def kernel(x_hbm, go_hbm, wd_hbm, wu_hbm, out_hbm, dx_hbm, dwd_hbm, dwu_hbm,
               xb, gb, wd_v, wu_v, dwd_v, dwu_v, rsem, wsem, ssem):
        buf = (xb, gb)
        src = (x_hbm, go_hbm)
        dst = (out_hbm, dx_hbm)

        def rows_at(start, n):
            if not isinstance(start, int):
                start = pl.multiple_of(start, PIECE)
            return pl.ds(start, n)

        segs0 = tuple(jnp.int32(p * inv_nv % SET_SEGS) for p in range(SET_SEGS))

        def rotate(segs):
            return segs[-1:] + segs[:-1]

        def chunks(s, v, segs):
            rows = rows_at(v * CH, CH)
            return [((segs[p] + s * SET_SEGS, rows, slice(None)),
                     [(p * (CH // SUB) + i) // WB for i in range(CH // SUB)])
                    for p in range(SET_SEGS)]

        def tiles(v):
            return [v[i * SUB:(i + 1) * SUB] for i in range(CH // SUB)]

        def read_copy(st, j, n=1, sem=None):
            a, s = st
            idx = (pl.ds(s * SET_SEGS, SET_SEGS), rows_at(j * PIECE, n * PIECE))
            sem = 3 * a + s if sem is None else sem
            return pltpu.make_async_copy(src[a].at[idx], buf[a].at[idx], rsem.at[sem])

        def read_steps(i0, i1, body=None, acc=0):
            cuts = {i0, i1} | {p * NP for p in range(3)} | {p * NP - SKEW for p in range(3)}
            cuts = sorted(c for c in cuts if i0 <= c <= i1)
            assert body is None or len(cuts) == 2
            carry = 0 if body is None else (segs0, acc)
            for lo, hi in zip(cuts[:-1], cuts[1:]):
                def step(i, c, ph=lo // NP, pw=(lo + SKEW) // NP):
                    read_copy(HIGH_SETS[ph], i - ph * NP).start(priority=0)
                    read_copy(LOW_SETS[pw], i + SKEW - pw * NP).start(priority=1)
                    return c if body is None else body(i - i0, c)

                carry = lax.fori_loop(lo, hi, step, carry)
            return None if body is None else carry[1]

        last_sets = (HIGH_SETS[2], LOW_SETS[2])
        shared = NP - SKEW // 2
        drain = [(last_sets[u % 2], shared + u // 2) for u in range(SKEW)]
        marker = drain[SKEW - LEAD]
        marker_copy = read_copy(*marker, sem=6)

        def read_drain():
            for u, piece in enumerate(drain):
                read_copy(last_sets[0], shared - SKEW + u).start(priority=0)
                (marker_copy if piece == marker else read_copy(*piece)).start(priority=1)

        def write_block(a, k, ready, body=None, acc=0):
            s0, n = sum(WRITE_BLOCKS[:k]), WRITE_BLOCKS[k]
            assert s0 + n <= (ready + (body is not None)) * SET_SEGS

            def step(v, c):
                if body is not None:
                    c = body(ready, v, c)
                for u in range(CH // PIECE):
                    idx = (pl.ds(s0, n), rows_at(v * CH + u * PIECE, PIECE))
                    pltpu.make_async_copy(buf[a].at[idx], dst[a].at[idx], wsem.at[a]).start()
                return c

            carry = lax.fori_loop(0, NV, step, 0 if body is None else (segs0, acc))
            return None if body is None else carry[1]

        def diag():
            return (lax.broadcasted_iota(jnp.int32, (C, C), 0)
                    == lax.broadcasted_iota(jnp.int32, (C, C), 1))

        def acc_to_row(acc):
            col = jnp.sum(jnp.concatenate(acc, axis=0), axis=1, keepdims=True)
            return jnp.sum(jnp.where(diag(), col, 0.0), axis=0, keepdims=True)

        def row_to_tiles(row):
            col = jnp.sum(jnp.where(diag(), row, 0.0), axis=1, keepdims=True)
            full = jnp.broadcast_to(col, (C, LANES))
            return tuple(full[i * SUB:(i + 1) * SUB] for i in range(CB))

        zeros = tuple(jnp.zeros((SUB, LANES), jnp.float32) for _ in range(CB))

        def sum_x(sets, v, c):
            segs, acc = c[0], list(c[1])
            for s in sets:
                for idx, cbs in chunks(s, v, segs):
                    for cb, t in zip(cbs, tiles(xb[idx].astype(jnp.float32))):
                        acc[cb] = acc[cb] + t
            return rotate(segs), tuple(acc)

        def sum_x_last(k, c):
            for u in range(4):
                c = sum_x((2,), 4 * k + u, c)
            return c

        for j in range(SKEW):
            read_copy(LOW_SETS[0], j).start(priority=1)
        read_steps(0, NP)
        wd_copy = pltpu.make_async_copy(wd_hbm, wd_v, ssem.at[0])
        wu_copy = pltpu.make_async_copy(wu_hbm, wu_v, ssem.at[1])
        wd_copy.start()
        wu_copy.start()
        i = NP + SETTLE
        read_steps(NP, i)
        read_copy(HIGH_SETS[0], 0, NP).wait()
        read_copy(LOW_SETS[0], 0, NP).wait()
        acc = read_steps(i, i + NV, lambda v, c: sum_x((0, 1), v, c), zeros)
        read_steps(i + NV, 2 * NP + SETTLE)

        i = 2 * NP + SETTLE
        read_copy(HIGH_SETS[1], 0, NP).wait()
        read_copy(LOW_SETS[1], 0, NP).wait()
        acc = read_steps(i, i + NV // 4, sum_x_last, acc)
        i += NV // 4

        wd_copy.wait()
        wu_copy.wait()
        wd = wd_v[...].astype(jnp.float32)
        wu = wu_v[...].astype(jnp.float32)
        s_row = acc_to_row(acc) * inv_n
        z1 = jnp.sum(wd * s_row, axis=1, keepdims=True)
        sig1 = jax.nn.sigmoid(z1)
        hid = z1 * sig1
        gate = jax.nn.sigmoid(jnp.sum(wu * hid, axis=0, keepdims=True))
        gate_t = row_to_tiles(gate)

        def scale_x(s, v, c):
            segs, acc = c[0], list(c[1])
            todo = chunks(s, v, segs)
            for g in range(0, SET_SEGS, PRELOAD):
                for idx, cbs, xr in [(idx, cbs, xb[idx]) for idx, cbs in todo[g:g + PRELOAD]]:
                    xv = xr.astype(jnp.float32)
                    for cb, t in zip(cbs, tiles(xv * gb[idx].astype(jnp.float32))):
                        acc[cb] = acc[cb] + t
                    outs = [t * gate_t[cb] for cb, t in zip(cbs, tiles(xv))]
                    xb[idx] = jnp.concatenate(outs, axis=0).astype(xb.dtype)
            return rotate(segs), tuple(acc)

        acc = read_steps(i, i + NV, lambda v, c: scale_x(0, v, c), zeros)
        read_steps(i + NV, 2 * NP + shared - SKEW)
        read_drain()

        marker_copy.wait()
        write_block(0, 0, 1)
        for st in last_sets:
            if st == marker[0]:
                read_copy(st, 0, marker[1]).wait()
                read_copy(st, marker[1] + 1, NP - marker[1] - 1).wait()
            else:
                read_copy(st, 0, NP).wait()
        acc = write_block(0, 1, 1, scale_x, acc)
        acc = write_block(0, 2, 2, scale_x, acc)

        dz2 = acc_to_row(acc) * gate * (1.0 - gate)
        dwu_v[...] = (hid * dz2).astype(dwu_v.dtype)
        dh = jnp.sum(wu * dz2, axis=1, keepdims=True)
        dz1 = dh * (sig1 * (1.0 + z1 * (1.0 - sig1)))
        dwd_v[...] = (dz1 * s_row).astype(dwd_v.dtype)
        ds_t = row_to_tiles(jnp.sum(wd * dz1, axis=0, keepdims=True) * inv_n)
        dwd_copy = pltpu.make_async_copy(dwd_v, dwd_hbm, ssem.at[2])
        dwu_copy = pltpu.make_async_copy(dwu_v, dwu_hbm, ssem.at[3])
        dwd_copy.start()
        dwu_copy.start()
        write_block(0, 3, 3)

        def grad_x(s, v, c):
            for idx, cbs, gr in [(idx, cbs, gb[idx]) for idx, cbs in chunks(s, v, c[0])]:
                outs = [t * gate_t[cb] + ds_t[cb]
                        for cb, t in zip(cbs, tiles(gr.astype(jnp.float32)))]
                gb[idx] = jnp.concatenate(outs, axis=0).astype(gb.dtype)
            return rotate(c[0]), c[1]

        for k in range(3):
            write_block(1, k, k, grad_x)
        write_block(1, 3, 3)

        dwd_copy.wait()
        dwu_copy.wait()
        pltpu.make_async_copy(xb, out_hbm, wsem.at[0]).wait()
        pltpu.make_async_copy(gb, dx_hbm, wsem.at[1]).wait()

    return kernel


@jax.jit
def pallas_standalone__channel_attn_se__vision_kernel(
    x: jax.Array,
    w_down: jax.Array,
    w_up: jax.Array,
    grad_out: jax.Array,
):
    B, H, W, C = x.shape
    R = w_down.shape[1]
    assert B == 1
    WB = W // LANES
    seg_shape = (H * C * WB // SEG, SEG, LANES)

    def to_segments(a):
        a = jnp.transpose(a, (0, 1, 3, 2)).reshape(H * C // SUB, SUB, WB, LANES)
        return jnp.transpose(a, (0, 2, 1, 3)).reshape(seg_shape)

    def from_segments(a):
        a = a.reshape(H * C // SUB, WB, SUB, LANES)
        a = jnp.transpose(a, (0, 2, 1, 3)).reshape(B, H, C, W)
        return jnp.transpose(a, (0, 1, 3, 2))

    any_spec = pl.BlockSpec(memory_space=pl.ANY)
    out, dx, dwd_t, dwu = pl.pallas_call(
        _make_kernel(H, W, C),
        in_specs=[any_spec] * 4,
        out_specs=[any_spec] * 4,
        out_shape=[
            jax.ShapeDtypeStruct(seg_shape, x.dtype),
            jax.ShapeDtypeStruct(seg_shape, x.dtype),
            jax.ShapeDtypeStruct((R, C), w_down.dtype),
            jax.ShapeDtypeStruct((R, C), w_up.dtype),
        ],
        scratch_shapes=[
            pltpu.VMEM(seg_shape, x.dtype),
            pltpu.VMEM(seg_shape, grad_out.dtype),
            pltpu.VMEM((R, C), w_down.dtype),
            pltpu.VMEM((R, C), w_up.dtype),
            pltpu.VMEM((R, C), w_down.dtype),
            pltpu.VMEM((R, C), w_up.dtype),
            pltpu.SemaphoreType.DMA((7,)),
            pltpu.SemaphoreType.DMA((2,)),
            pltpu.SemaphoreType.DMA((4,)),
        ],
        compiler_params=pltpu.CompilerParams(
            vmem_limit_bytes=80 * 1024 * 1024,
            disable_semaphore_checks=True,
            disable_bounds_checks=True,
        ),
    )(to_segments(x), to_segments(grad_out), w_down.T, w_up)
    return from_segments(out), from_segments(dx), dwd_t.T, dwu
```

```python
import math

import jax
import jax.numpy as jnp
from jax import lax
import jax.experimental.pallas as pl
import jax.experimental.pallas.tpu as pltpu

LANES = 128
SUB = 8

SEG = 4096
PIECE = 16
SKEW = 26
SETTLE = 36
LEAD = 13
PRELOAD = 5
WRITE_BLOCKS = (6, 7, 7, 7)
HIGH_SETS = ((0, 0), (1, 0), (1, 1))
LOW_SETS = ((0, 1), (0, 2), (1, 2))


def _make_kernel(H, W, C):
    WB = W // LANES
    CB = C // SUB
    ROWS = C * WB
    NSEG = H * ROWS // SEG
    SET_SEGS = NSEG // 3
    CH = math.gcd(SEG, ROWS)
    NV = SEG // CH
    NP = SEG // PIECE
    assert W % LANES == 0 and C % SUB == 0 and 3 * SET_SEGS * SEG == H * ROWS
    assert SET_SEGS * CH == ROWS and CH % PIECE == 0 and PIECE % (2 * SUB) == 0
    assert sum(WRITE_BLOCKS) == NSEG and len(WRITE_BLOCKS) == 4 and NV % 4 == 0
    inv_nv = pow(NV, -1, SET_SEGS)
    inv_n = 1.0 / (H * W)

    def kernel(x_hbm, go_hbm, wd_hbm, wu_hbm, out_hbm, dx_hbm, dwd_hbm, dwu_hbm,
               xb, gb, wd_v, wu_v, dwd_v, dwu_v, rsem, wsem, ssem):
        buf = (xb, gb)
        src = (x_hbm, go_hbm)
        dst = (out_hbm, dx_hbm)

        def rows_at(start, n):
            if not isinstance(start, int):
                start = pl.multiple_of(start, PIECE)
            return pl.ds(start, n)

        segs0 = tuple(jnp.int32(p * inv_nv % SET_SEGS) for p in range(SET_SEGS))

        def rotate(segs):
            return segs[-1:] + segs[:-1]

        def chunks(s, v, segs):
            rows = rows_at(v * CH, CH)
            return [((segs[p] + s * SET_SEGS, rows, slice(None)),
                     [(p * (CH // SUB) + i) // WB for i in range(CH // SUB)])
                    for p in range(SET_SEGS)]

        def tiles(v):
            return [v[i * SUB:(i + 1) * SUB] for i in range(CH // SUB)]

        def read_copy(st, j, n=1, sem=None):
            a, s = st
            idx = (pl.ds(s * SET_SEGS, SET_SEGS), rows_at(j * PIECE, n * PIECE))
            sem = 3 * a + s if sem is None else sem
            return pltpu.make_async_copy(src[a].at[idx], buf[a].at[idx], rsem.at[sem])

        def read_steps(i0, i1, body=None, acc=0):
            cuts = {i0, i1} | {p * NP for p in range(3)} | {p * NP - SKEW for p in range(3)}
            cuts = sorted(c for c in cuts if i0 <= c <= i1)
            assert body is None or len(cuts) == 2
            carry = 0 if body is None else (segs0, acc)
            for lo, hi in zip(cuts[:-1], cuts[1:]):
                def step(i, c, ph=lo // NP, pw=(lo + SKEW) // NP):
                    read_copy(HIGH_SETS[ph], i - ph * NP).start(priority=0)
                    read_copy(LOW_SETS[pw], i + SKEW - pw * NP).start(priority=1)
                    return c if body is None else body(i - i0, c)

                carry = lax.fori_loop(lo, hi, step, carry)
            return None if body is None else carry[1]

        last_sets = (HIGH_SETS[2], LOW_SETS[2])
        shared = NP - SKEW // 2
        drain = [(last_sets[u % 2], shared + u // 2) for u in range(SKEW)]
        marker = drain[SKEW - LEAD]
        marker_copy = read_copy(*marker, sem=6)

        def read_drain():
            for u, piece in enumerate(drain):
                read_copy(last_sets[0], shared - SKEW + u).start(priority=0)
                (marker_copy if piece == marker else read_copy(*piece)).start(priority=1)

        def write_copy(b, start, n):
            a, k = divmod(b, len(WRITE_BLOCKS))
            idx = (pl.ds(sum(WRITE_BLOCKS[:k]), WRITE_BLOCKS[k]), rows_at(start, n))
            return pltpu.make_async_copy(buf[a].at[idx], dst[a].at[idx], wsem.at[b])

        def write_block(b, ready, body=None, acc=0):
            k = b % len(WRITE_BLOCKS)
            assert sum(WRITE_BLOCKS[:k + 1]) <= (ready + (body is not None)) * SET_SEGS

            def step(v, c):
                if body is not None:
                    c = body(ready, v, c)
                for u in range(CH // PIECE):
                    write_copy(b, v * CH + u * PIECE, PIECE).start()
                return c

            carry = lax.fori_loop(0, NV, step, 0 if body is None else (segs0, acc))
            if b > 0:
                write_copy(b - 1, 0, SEG).wait()
            return None if body is None else carry[1]

        def diag():
            return (lax.broadcasted_iota(jnp.int32, (C, C), 0)
                    == lax.broadcasted_iota(jnp.int32, (C, C), 1))

        def acc_to_row(acc):
            col = jnp.sum(jnp.concatenate(acc, axis=0), axis=1, keepdims=True)
            return jnp.sum(jnp.where(diag(), col, 0.0), axis=0, keepdims=True)

        def row_to_tiles(row):
            col = jnp.sum(jnp.where(diag(), row, 0.0), axis=1, keepdims=True)
            full = jnp.broadcast_to(col, (C, LANES))
            return tuple(full[i * SUB:(i + 1) * SUB] for i in range(CB))

        zeros = tuple(jnp.zeros((SUB, LANES), jnp.float32) for _ in range(CB))

        def sum_x(sets, v, c):
            segs, acc = c[0], list(c[1])
            for s in sets:
                for idx, cbs in chunks(s, v, segs):
                    for cb, t in zip(cbs, tiles(xb[idx].astype(jnp.float32))):
                        acc[cb] = acc[cb] + t
            return rotate(segs), tuple(acc)

        def sum_x_last(k, c):
            for u in range(4):
                c = sum_x((2,), 4 * k + u, c)
            return c

        for j in range(SKEW):
            read_copy(LOW_SETS[0], j).start(priority=1)
        read_steps(0, NP)
        wd_copy = pltpu.make_async_copy(wd_hbm, wd_v, ssem.at[0])
        wu_copy = pltpu.make_async_copy(wu_hbm, wu_v, ssem.at[1])
        wd_copy.start()
        wu_copy.start()
        i = NP + SETTLE
        read_steps(NP, i)
        read_copy(HIGH_SETS[0], 0, NP).wait()
        read_copy(LOW_SETS[0], 0, NP).wait()
        acc = read_steps(i, i + NV, lambda v, c: sum_x((0, 1), v, c), zeros)
        read_steps(i + NV, 2 * NP + SETTLE)

        i = 2 * NP + SETTLE
        read_copy(HIGH_SETS[1], 0, NP).wait()
        read_copy(LOW_SETS[1], 0, NP).wait()
        acc = read_steps(i, i + NV // 4, sum_x_last, acc)
        i += NV // 4

        wd_copy.wait()
        wu_copy.wait()
        wd = wd_v[...].astype(jnp.float32)
        wu = wu_v[...].astype(jnp.float32)
        s_row = acc_to_row(acc) * inv_n
        z1 = jnp.sum(wd * s_row, axis=1, keepdims=True)
        sig1 = jax.nn.sigmoid(z1)
        hid = z1 * sig1
        gate = jax.nn.sigmoid(jnp.sum(wu * hid, axis=0, keepdims=True))
        gate_t = row_to_tiles(gate)

        def scale_x(s, v, c):
            segs, acc = c[0], list(c[1])
            todo = chunks(s, v, segs)
            for g in range(0, SET_SEGS, PRELOAD):
                for idx, cbs, xr in [(idx, cbs, xb[idx]) for idx, cbs in todo[g:g + PRELOAD]]:
                    xv = xr.astype(jnp.float32)
                    for cb, t in zip(cbs, tiles(xv * gb[idx].astype(jnp.float32))):
                        acc[cb] = acc[cb] + t
                    outs = [t * gate_t[cb] for cb, t in zip(cbs, tiles(xv))]
                    xb[idx] = jnp.concatenate(outs, axis=0).astype(xb.dtype)
            return rotate(segs), tuple(acc)

        acc = read_steps(i, i + NV, lambda v, c: scale_x(0, v, c), zeros)
        read_steps(i + NV, 2 * NP + shared - SKEW)
        read_drain()

        marker_copy.wait()
        write_block(0, 1)
        for st in last_sets:
            if st == marker[0]:
                read_copy(st, 0, marker[1]).wait()
                read_copy(st, marker[1] + 1, NP - marker[1] - 1).wait()
            else:
                read_copy(st, 0, NP).wait()
        acc = write_block(1, 1, scale_x, acc)
        acc = write_block(2, 2, scale_x, acc)

        dz2 = acc_to_row(acc) * gate * (1.0 - gate)
        dwu_v[...] = (hid * dz2).astype(dwu_v.dtype)
        dh = jnp.sum(wu * dz2, axis=1, keepdims=True)
        dz1 = dh * (sig1 * (1.0 + z1 * (1.0 - sig1)))
        dwd_v[...] = (dz1 * s_row).astype(dwd_v.dtype)
        ds_t = row_to_tiles(jnp.sum(wd * dz1, axis=0, keepdims=True) * inv_n)
        dwd_copy = pltpu.make_async_copy(dwd_v, dwd_hbm, ssem.at[2])
        dwu_copy = pltpu.make_async_copy(dwu_v, dwu_hbm, ssem.at[3])
        dwd_copy.start()
        dwu_copy.start()
        write_block(3, 3)

        def grad_x(s, v, c):
            for idx, cbs, gr in [(idx, cbs, gb[idx]) for idx, cbs in chunks(s, v, c[0])]:
                outs = [t * gate_t[cb] + ds_t[cb]
                        for cb, t in zip(cbs, tiles(gr.astype(jnp.float32)))]
                gb[idx] = jnp.concatenate(outs, axis=0).astype(gb.dtype)
            return rotate(c[0]), c[1]

        for s in range(3):
            write_block(4 + s, s, grad_x)
        write_block(7, 3)

        dwd_copy.wait()
        dwu_copy.wait()
        write_copy(7, 0, SEG).wait()

    return kernel


@jax.jit
def pallas_standalone__channel_attn_se__vision_kernel(
    x: jax.Array,
    w_down: jax.Array,
    w_up: jax.Array,
    grad_out: jax.Array,
):
    B, H, W, C = x.shape
    R = w_down.shape[1]
    assert B == 1
    WB = W // LANES
    seg_shape = (H * C * WB // SEG, SEG, LANES)

    def to_segments(a):
        a = jnp.transpose(a, (0, 1, 3, 2)).reshape(H * C // SUB, SUB, WB, LANES)
        return jnp.transpose(a, (0, 2, 1, 3)).reshape(seg_shape)

    def from_segments(a):
        a = a.reshape(H * C // SUB, WB, SUB, LANES)
        a = jnp.transpose(a, (0, 2, 1, 3)).reshape(B, H, C, W)
        return jnp.transpose(a, (0, 1, 3, 2))

    any_spec = pl.BlockSpec(memory_space=pl.ANY)
    out, dx, dwd_t, dwu = pl.pallas_call(
        _make_kernel(H, W, C),
        in_specs=[any_spec] * 4,
        out_specs=[any_spec] * 4,
        out_shape=[
            jax.ShapeDtypeStruct(seg_shape, x.dtype),
            jax.ShapeDtypeStruct(seg_shape, x.dtype),
            jax.ShapeDtypeStruct((R, C), w_down.dtype),
            jax.ShapeDtypeStruct((R, C), w_up.dtype),
        ],
        scratch_shapes=[
            pltpu.VMEM(seg_shape, x.dtype),
            pltpu.VMEM(seg_shape, grad_out.dtype),
            pltpu.VMEM((R, C), w_down.dtype),
            pltpu.VMEM((R, C), w_up.dtype),
            pltpu.VMEM((R, C), w_down.dtype),
            pltpu.VMEM((R, C), w_up.dtype),
            pltpu.SemaphoreType.DMA((7,)),
            pltpu.SemaphoreType.DMA((2 * len(WRITE_BLOCKS),)),
            pltpu.SemaphoreType.DMA((4,)),
        ],
        compiler_params=pltpu.CompilerParams(
            vmem_limit_bytes=80 * 1024 * 1024,
            disable_semaphore_checks=True,
            disable_bounds_checks=True,
        ),
    )(to_segments(x), to_segments(grad_out), w_down.T, w_up)
    return from_segments(out), from_segments(dx), dwd_t.T, dwu
```
